```python
import os as _os
_os.environ.setdefault("JAX_PLATFORMS", "cpu")
import jax
import jax.numpy as jnp

def _softmax(x, axis=-1):
    return jax.nn.softmax(x, axis=axis)
def _gelu(x):
    return jax.nn.gelu(x, approximate=True)
def _silu(x):
    return jax.nn.silu(x)
def _sigmoid(x):
    return jax.nn.sigmoid(x)
def _layernorm(x, axis=-1, eps=1e-5):
    m = jnp.mean(x, axis=axis, keepdims=True)
    v = jnp.var(x, axis=axis, keepdims=True)
    return (x - m) / jnp.sqrt(v + eps)
def _scatter_add(tgt, idx, src, axis=0):
    return tgt.at[idx].add(src)
def _segment_sum(src, seg, n):
    return jax.ops.segment_sum(src, seg, n)
class _Rng:
    def __init__(self, key):
        self._k = key
    def _next(self):
        self._k, sub = jax.random.split(self._k)
        return sub
    def normal(self, shape):
        return jax.random.normal(self._next(), shape, dtype=jnp.bfloat16)
    def randint(self, lo, hi, shape):
        return jax.random.randint(self._next(), shape, lo, hi, dtype=jnp.int32)
    def uniform(self, shape, lo=0.0, hi=1.0):
        return jax.random.uniform(self._next(), shape, jnp.bfloat16, lo, hi)
    def permutation(self, n):
        return jax.random.permutation(self._next(), n)


kernel_name = 'concat_heads__mha_block_cached__mha_block_cached__near_ridge'

def setup_inputs():
    _rng = _Rng(jax.random.key(int.from_bytes(__import__("os").urandom(4), "little")))
    _w = (lambda a: (lambda t: t.astype(jnp.bfloat16) if jnp.issubdtype(t.dtype, jnp.floating) else t)(jnp.asarray(a)))
    def _A_setup():
        B, Sq, D = 32, 32, 640
        H, Sk, Dh = 32, 32, 128
        return {
            "x": _w((lambda *s: _rng.normal(s) * 0.8)(B, Sq, D)),
            "k_cache": _w((lambda *s: _rng.normal(s) * 0.8)(B, H, Sk, Dh)),
            "v_cache": _w((lambda *s: _rng.normal(s) * 0.05)(B, H, Sk, Dh)),
            "wq": _w((lambda *s: _rng.normal(s) * 0.8)(D, H * Dh) * (D ** -0.5)),
            "wo": _w((lambda *s: _rng.normal(s) * 0.05)(H * Dh, D) * ((H * Dh) ** -0.5)),
        }
    _A_in = _A_setup()

    def _B_setup():
        B, Sq, D = 32, 32, 640
        H, Sk, Dh = 32, 32, 128
        return {
            "x": _w((lambda *s: _rng.normal(s) * 0.8)(B, Sq, D)),
            "k_cache": _w((lambda *s: _rng.normal(s) * 0.8)(B, H, Sk, Dh)),
            "v_cache": _w((lambda *s: _rng.normal(s) * 0.05)(B, H, Sk, Dh)),
            "wq": _w((lambda *s: _rng.normal(s) * 0.8)(D, H * Dh) * (D ** -0.5)),
            "wo": _w((lambda *s: _rng.normal(s) * 0.05)(H * Dh, D) * ((H * Dh) ** -0.5)),
        }
    _B_in = _B_setup()

    return {
        "A_x": _A_in["x"],
        "A_k_cache": _A_in["k_cache"],
        "A_v_cache": _A_in["v_cache"],
        "A_wq": _A_in["wq"],
        "A_wo": _A_in["wo"],
        "B_x": _B_in["x"],
        "B_k_cache": _B_in["k_cache"],
        "B_v_cache": _B_in["v_cache"],
        "B_wq": _B_in["wq"],
        "B_wo": _B_in["wo"],
    }

def reference(A_x, A_k_cache, A_v_cache, A_wq, A_wo, B_x, B_k_cache, B_v_cache, B_wq, B_wo):
    def _A_ref(x, k_cache, v_cache, wq, wo):
        B, Sq, D = x.shape
        H, Dh = 32, 128
        q = (lambda x, *d: x.transpose(*d))((x @ wq).reshape(B, Sq, H, Dh), 0, 2, 1, 3)
        scores = jnp.einsum("bhqd,bhkd->bhqk", q, k_cache) * (Dh ** -0.5)
        p = _softmax(scores, axis=-1)
        o = jnp.einsum("bhqk,bhkd->bhqd", p, v_cache)
        return (lambda x, *d: x.transpose(*d))(o, 0, 2, 1, 3).reshape(B, Sq, H * Dh) @ wo

    def _B_ref(x, k_cache, v_cache, wq, wo):
        B, Sq, D = x.shape
        H, Dh = 32, 128
        q = (lambda x, *d: x.transpose(*d))((x @ wq).reshape(B, Sq, H, Dh), 0, 2, 1, 3)
        scores = jnp.einsum("bhqd,bhkd->bhqk", q, k_cache) * (Dh ** -0.5)
        p = _softmax(scores, axis=-1)
        o = jnp.einsum("bhqk,bhkd->bhqd", p, v_cache)
        return (lambda x, *d: x.transpose(*d))(o, 0, 2, 1, 3).reshape(B, Sq, H * Dh) @ wo

    a = _A_ref(A_x, A_k_cache, A_v_cache, A_wq, A_wo)
    b = _B_ref(B_x, B_k_cache, B_v_cache, B_wq, B_wo)
    return jnp.concatenate([a, b], axis=-1)
```

```python
import functools

import jax
import jax.numpy as jnp
from jax import lax
import jax.experimental.pallas as pl
import jax.experimental.pallas.tpu as pltpu

B, SQ, D = 32, 32, 640
H, SK, DH = 32, 32, 128
HG = 4
NG = H // HG
GW = HG * DH
M = B * SQ
NSTEPS = 2 * NG
SCALE = DH ** -0.5
UNROLL = 4


def _kernel(xa, ka, va, wqa, woa, xb, kb, vb, wqb, wob,
            o_ref,
            x_buf, wq_buf, wo_buf, k_buf, v_buf, q_scr, o_scr, acc, sems, xsems):
    s = pl.program_id(0)
    br = s // NG
    g = s % NG
    slot = s % 2
    refs = ((xa, ka, va, wqa, woa), (xb, kb, vb, wqb, wob))

    def copies(branch, grp, sl):
        _, k, v, wq, wo = refs[branch]
        off = pl.multiple_of(grp * GW, GW)
        return (
            pltpu.make_async_copy(wq.at[:, pl.ds(off, GW)], wq_buf.at[sl], sems.at[0, sl]),
            pltpu.make_async_copy(k.at[:, grp], k_buf.at[sl], sems.at[1, sl]),
            pltpu.make_async_copy(v.at[:, grp], v_buf.at[sl], sems.at[2, sl]),
            pltpu.make_async_copy(wo.at[pl.ds(off, GW), :], wo_buf.at[sl], sems.at[3, sl]),
        )

    def xcopy(branch):
        return pltpu.make_async_copy(refs[branch][0], x_buf.at[branch], xsems.at[branch])

    @pl.when(s == 0)
    def _():
        xcopy(0).start()
        for c in copies(0, 0, 0):
            c.start()

    nxt = s + 1
    for branch in range(2):
        @pl.when(jnp.logical_and(nxt < NSTEPS, nxt // NG == branch))
        def _():
            for c in copies(branch, nxt % NG, 1 - slot):
                c.start()

    @pl.when(s == NG - 2)
    def _():
        xcopy(1).start()

    def wait(idx):
        for branch in range(2):
            @pl.when(br == branch)
            def _():
                copies(branch, g, slot)[idx].wait()

    for branch in range(2):
        @pl.when(s == branch * NG)
        def _():
            xcopy(branch).wait()

    wait(0)
    q_scr[...] = jnp.dot(x_buf[br], wq_buf[slot],
                         preferred_element_type=jnp.float32).astype(jnp.bfloat16)

    wait(1)
    wait(2)

    row_h = lax.broadcasted_iota(jnp.int32, (HG * SQ, HG * SK), 0) // SQ
    col_h = lax.broadcasted_iota(jnp.int32, (HG * SQ, HG * SK), 1) // SK
    mask = row_h == col_h

    def attn(b, carry):
        r0 = pl.multiple_of(b * SQ, SQ)
        q = q_scr[pl.ds(r0, SQ), :]
        qs = jnp.concatenate([q[:, h * DH:(h + 1) * DH] for h in range(HG)], axis=0)
        k = k_buf[slot, b]
        v = v_buf[slot, b]
        sc = lax.dot_general(qs, k, (((1,), (1,)), ((), ())),
                             preferred_element_type=jnp.float32)
        sc = jnp.where(mask, sc, -jnp.inf)
        m = jnp.max(sc, axis=-1, keepdims=True)
        p = jnp.exp((sc - m) * SCALE)
        l = jnp.sum(p, axis=-1, keepdims=True)
        p = (p * (1.0 / l)).astype(jnp.bfloat16)
        o = jnp.dot(p, v, preferred_element_type=jnp.float32).astype(jnp.bfloat16)
        for h in range(HG):
            o_scr[pl.ds(r0, SQ), h * DH:(h + 1) * DH] = o[h * SQ:(h + 1) * SQ, :]
        return carry

    lax.fori_loop(0, B, attn, 0, unroll=UNROLL)

    wait(3)
    part = jnp.dot(o_scr[...], wo_buf[slot], preferred_element_type=jnp.float32)

    @pl.when(g == 0)
    def _():
        acc[...] = part

    @pl.when(g > 0)
    def _():
        acc[...] += part

    @pl.when(g == NG - 1)
    def _():
        o_ref[...] = acc[...].astype(o_ref.dtype)


@jax.jit
def pallas_concat_heads__mha_block_cached__mha_block_cached__near_ridge_kernel(
    A_x: jax.Array,
    A_k_cache: jax.Array,
    A_v_cache: jax.Array,
    A_wq: jax.Array,
    A_wo: jax.Array,
    B_x: jax.Array,
    B_k_cache: jax.Array,
    B_v_cache: jax.Array,
    B_wq: jax.Array,
    B_wo: jax.Array,
):
    def prep(x, k, v, wq, wo):
        return (x.reshape(M, D),
                k.reshape(B, NG, HG * SK, DH),
                v.reshape(B, NG, HG * SK, DH),
                wq, wo)

    args = prep(A_x, A_k_cache, A_v_cache, A_wq, A_wo) + prep(B_x, B_k_cache, B_v_cache, B_wq, B_wo)
    bf = jnp.bfloat16
    out = pl.pallas_call(
        _kernel,
        grid=(NSTEPS,),
        in_specs=[pl.BlockSpec(memory_space=pl.ANY)] * 10,
        out_specs=pl.BlockSpec((M, D), lambda s: (0, s // NG)),
        out_shape=jax.ShapeDtypeStruct((M, 2 * D), bf),
        scratch_shapes=[
            pltpu.VMEM((2, M, D), bf),
            pltpu.VMEM((2, D, GW), bf),
            pltpu.VMEM((2, GW, D), bf),
            pltpu.VMEM((2, B, HG * SK, DH), bf),
            pltpu.VMEM((2, B, HG * SK, DH), bf),
            pltpu.VMEM((M, GW), bf),
            pltpu.VMEM((M, GW), bf),
            pltpu.VMEM((M, D), jnp.float32),
            pltpu.SemaphoreType.DMA((4, 2)),
            pltpu.SemaphoreType.DMA((2,)),
        ],
        compiler_params=pltpu.CompilerParams(
            dimension_semantics=("arbitrary",),
            vmem_limit_bytes=64 * 1024 * 1024,
        ),
    )(*args)
    return out.reshape(B, SQ, 2 * D)
```

```python
import functools

import jax
import jax.numpy as jnp
from jax import lax
import jax.experimental.pallas as pl
import jax.experimental.pallas.tpu as pltpu

B, SQ, D = 32, 32, 640
H, SK, DH = 32, 32, 128
HG = 4
NG = H // HG
GW = HG * DH
M = B * SQ
NSTEPS = 2 * NG
SCALE = DH ** -0.5
XCH = 4
XR = M // XCH
NCHUNK = 1


def _kernel(xa, ka, va, wqa, woa, xb, kb, vb, wqb, wob,
            o_ref,
            x_buf, wq_buf, wo_buf, k_buf, v_buf, q_scr, o_scr, acc, s_scr, p_scr, sems, xsems):
    s = pl.program_id(0)
    br = s // NG
    g = s % NG
    slot = s % 2
    refs = ((xa, ka, va, wqa, woa), (xb, kb, vb, wqb, wob))

    def cp(idx, branch, grp, sl):
        _, k, v, wq, wo = refs[branch]
        off = pl.multiple_of(grp * GW, GW)
        if idx == 0:
            return pltpu.make_async_copy(wq.at[:, pl.ds(off, GW)], wq_buf.at[sl], sems.at[0, sl])
        if idx == 1:
            return pltpu.make_async_copy(k.at[:, grp], k_buf.at[sl], sems.at[1, sl])
        if idx == 2:
            return pltpu.make_async_copy(v.at[:, grp], v_buf.at[sl], sems.at[2, sl])
        return pltpu.make_async_copy(wo.at[pl.ds(off, GW), :], wo_buf.at[sl], sems.at[3, sl])

    def xcopy(branch):
        return pltpu.make_async_copy(refs[branch][0], x_buf.at[branch], xsems.at[XCH])

    def xchunk(c):
        return pltpu.make_async_copy(xa.at[pl.ds(c * XR, XR), :], x_buf.at[0, pl.ds(c * XR, XR), :],
                                     xsems.at[c])

    def for_step(t, idx, op):
        for branch in range(2):
            @pl.when(jnp.logical_and(t < NSTEPS, t // NG == branch))
            def _():
                c = cp(idx, branch, t % NG, t % 2)
                c.start() if op == "start" else c.wait()

    def qproj_rows(t_br, t_slot, r0, nrows):
        q_scr[pl.ds(r0, nrows), :] = jnp.dot(
            x_buf[t_br, pl.ds(r0, nrows), :], wq_buf[t_slot],
            preferred_element_type=jnp.float32).astype(jnp.bfloat16)

    @pl.when(s == 0)
    def _():
        with jax.named_scope("pro"):
            cp(0, 0, 0, 0).start()
            xchunk(0).start()
            cp(0, 0, 0, 0).wait()
            xchunk(0).wait()
            for c in range(1, XCH):
                xchunk(c).start()
            later = [cp(1, 0, 0, 0), cp(0, 0, 1, 1), cp(2, 0, 0, 0), cp(3, 0, 0, 0)]
            for c in range(XCH):
                if c > 0:
                    xchunk(c).wait()
                    later[c - 1].start()
                qproj_rows(0, 0, c * XR, XR)
            for l in later[XCH - 1:]:
                l.start()

    for_step(s + 2, 0, "start")
    for idx in (1, 2, 3):
        for_step(s + 1, idx, "start")

    @pl.when(s == NG - 3)
    def _():
        xcopy(1).start()

    row_h = lax.broadcasted_iota(jnp.int32, (HG * SQ, HG * SK), 0) // SQ
    col_h = lax.broadcasted_iota(jnp.int32, (HG * SQ, HG * SK), 1) // SK
    mask = row_h == col_h

    for_step(s, 1, "wait")
    with jax.named_scope("qk"):
        for b in range(B):
            q = q_scr[b * SQ:(b + 1) * SQ, :]
            qs = jnp.concatenate([q[:, h * DH:(h + 1) * DH] for h in range(HG)], axis=0)
            s_scr[b] = lax.dot_general(qs, k_buf[slot, b], (((1,), (1,)), ((), ())),
                                       preferred_element_type=jnp.float32)

    def softmax_b(b):
        sc = jnp.where(mask, s_scr[b], -jnp.inf)
        m = jnp.max(sc, axis=-1, keepdims=True)
        p = jnp.exp((sc - m) * SCALE)
        l = jnp.sum(p, axis=-1, keepdims=True)
        r = pl.reciprocal(l, approx=True)
        r = r * (2.0 - l * r)
        p_scr[b] = (p * r).astype(jnp.bfloat16)

    for_step(s + 1, 0, "wait")

    @pl.when(s == NG - 1)
    def _():
        xcopy(1).wait()

    with jax.named_scope("smq"):
        @pl.when(s < NSTEPS - 1)
        def _():
            nb = B // NCHUNK
            for c in range(NCHUNK):
                for b in range(c * nb, (c + 1) * nb):
                    softmax_b(b)
                qproj_rows((s + 1) // NG, (s + 1) % 2, c * nb * SQ, nb * SQ)

        @pl.when(s == NSTEPS - 1)
        def _():
            for b in range(B):
                softmax_b(b)

    for_step(s, 2, "wait")
    with jax.named_scope("pv"):
        for b in range(B):
            o = jnp.dot(p_scr[b], v_buf[slot, b], preferred_element_type=jnp.float32).astype(jnp.bfloat16)
            for h in range(HG):
                o_scr[b * SQ:(b + 1) * SQ, h * DH:(h + 1) * DH] = o[h * SQ:(h + 1) * SQ, :]

    for_step(s, 3, "wait")
    with jax.named_scope("oproj"):
        @pl.when(g < NG - 1)
        def _():
            prev = jnp.where(g > 0, acc[...], 0.0)
            acc[...] = prev + jnp.dot(o_scr[...], wo_buf[slot], preferred_element_type=jnp.float32)

        @pl.when(g == NG - 1)
        def _():
            o_ref[...] = (acc[...] + jnp.dot(o_scr[...], wo_buf[slot], preferred_element_type=jnp.float32)
                          ).astype(o_ref.dtype)


@jax.jit
def pallas_concat_heads__mha_block_cached__mha_block_cached__near_ridge_kernel(
    A_x: jax.Array,
    A_k_cache: jax.Array,
    A_v_cache: jax.Array,
    A_wq: jax.Array,
    A_wo: jax.Array,
    B_x: jax.Array,
    B_k_cache: jax.Array,
    B_v_cache: jax.Array,
    B_wq: jax.Array,
    B_wo: jax.Array,
):
    def prep(x, k, v, wq, wo):
        return (x.reshape(M, D),
                k.reshape(B, NG, HG * SK, DH),
                v.reshape(B, NG, HG * SK, DH),
                wq, wo)

    args = prep(A_x, A_k_cache, A_v_cache, A_wq, A_wo) + prep(B_x, B_k_cache, B_v_cache, B_wq, B_wo)
    bf = jnp.bfloat16
    out = pl.pallas_call(
        _kernel,
        grid=(NSTEPS,),
        in_specs=[pl.BlockSpec(memory_space=pl.ANY)] * 10,
        out_specs=pl.BlockSpec((M, D), lambda s: (0, s // NG)),
        out_shape=jax.ShapeDtypeStruct((M, 2 * D), bf),
        scratch_shapes=[
            pltpu.VMEM((2, M, D), bf),
            pltpu.VMEM((2, D, GW), bf),
            pltpu.VMEM((2, GW, D), bf),
            pltpu.VMEM((2, B, HG * SK, DH), bf),
            pltpu.VMEM((2, B, HG * SK, DH), bf),
            pltpu.VMEM((M, GW), bf),
            pltpu.VMEM((M, GW), bf),
            pltpu.VMEM((M, D), jnp.float32),
            pltpu.VMEM((B, HG * SQ, HG * SK), jnp.float32),
            pltpu.VMEM((B, HG * SQ, HG * SK), bf),
            pltpu.SemaphoreType.DMA((4, 2)),
            pltpu.SemaphoreType.DMA((XCH + 1,)),
        ],
        compiler_params=pltpu.CompilerParams(
            dimension_semantics=("arbitrary",),
            vmem_limit_bytes=64 * 1024 * 1024,
        ),
    )(*args)
    return out.reshape(B, SQ, 2 * D)
```

```python
import jax
import jax.numpy as jnp
from jax import lax
import jax.experimental.pallas as pl
import jax.experimental.pallas.tpu as pltpu

B, SQ, D = 32, 32, 640
H, SK, DH = 32, 32, 128
HG = 4
NG = H // HG
GW = HG * DH
M = B * SQ
NSTEPS = 2 * NG
SCALE = DH ** -0.5
XCH = 4
XR = M // XCH
OCH = 4
OR = M // OCH


def _kernel(xa, ka, va, wqa, woa, xb, kb, vb, wqb, wob,
            out_hbm,
            x_buf, wq_buf, wo_buf, k_buf, v_buf, q_scr, o_scr, acc, s_scr, p_scr, stage,
            sems, xsems, osems):
    s = pl.program_id(0)
    g = s % NG
    slot = s % 2
    refs = ((xa, ka, va, wqa, woa), (xb, kb, vb, wqb, wob))

    def cp(idx, branch, grp, sl):
        _, k, v, wq, wo = refs[branch]
        off = pl.multiple_of(grp * GW, GW)
        if idx == 0:
            return pltpu.make_async_copy(wq.at[:, pl.ds(off, GW)], wq_buf.at[sl], sems.at[0, sl])
        if idx == 1:
            return pltpu.make_async_copy(k.at[:, grp], k_buf.at[sl], sems.at[1, sl])
        if idx == 2:
            return pltpu.make_async_copy(v.at[:, grp], v_buf.at[sl], sems.at[2, sl])
        return pltpu.make_async_copy(wo.at[pl.ds(off, GW), :], wo_buf.at[sl], sems.at[3, sl])

    def xcopy_b():
        return pltpu.make_async_copy(xb, x_buf.at[1], xsems.at[XCH])

    def xchunk(c):
        return pltpu.make_async_copy(xa.at[pl.ds(c * XR, XR), :], x_buf.at[0, pl.ds(c * XR, XR), :],
                                     xsems.at[c])

    def ocopy_a():
        return pltpu.make_async_copy(stage.at[0], out_hbm.at[:, pl.ds(0, D)], osems.at[OCH])

    def ochunk_b(c):
        return pltpu.make_async_copy(stage.at[1, pl.ds(c * OR, OR), :],
                                     out_hbm.at[pl.ds(c * OR, OR), pl.ds(D, D)], osems.at[c])

    def for_step(t, idxs, op):
        for branch in range(2):
            @pl.when(jnp.logical_and(t < NSTEPS, t // NG == branch))
            def _():
                for idx in idxs:
                    c = cp(idx, branch, t % NG, t % 2)
                    c.start() if op == "start" else c.wait()

    def qproj_rows(t_br, t_slot, r0, nrows):
        q_scr[pl.ds(r0, nrows), :] = jnp.dot(
            x_buf[t_br, pl.ds(r0, nrows), :], wq_buf[t_slot],
            preferred_element_type=jnp.float32).astype(jnp.bfloat16)

    @pl.when(s == 0)
    def _():
        cp(0, 0, 0, 0).start()
        xchunk(0).start()
        cp(0, 0, 0, 0).wait()
        xchunk(0).wait()
        for c in range(1, XCH):
            xchunk(c).start()
        later = [cp(1, 0, 0, 0), cp(0, 0, 1, 1), cp(2, 0, 0, 0), cp(3, 0, 0, 0)]
        for c in range(XCH):
            if c > 0:
                xchunk(c).wait()
                later[c - 1].start()
            qproj_rows(0, 0, c * XR, XR)
        for l in later[XCH - 1:]:
            l.start()

    for_step(s, (1, 2, 3), "wait")
    for_step(s + 1, (0,), "wait")

    @pl.when(s == NG - 1)
    def _():
        xcopy_b().wait()

    row_h = lax.broadcasted_iota(jnp.int32, (HG * SQ, HG * SK), 0) // SQ
    col_h = lax.broadcasted_iota(jnp.int32, (HG * SQ, HG * SK), 1) // SK
    mask = row_h == col_h

    def oproj(sl, first):
        prev = jnp.where(first, 0.0, acc[...])
        acc[...] = prev + jnp.dot(o_scr[sl], wo_buf[sl], preferred_element_type=jnp.float32)

    def step_body(kind):
        if kind != "last":
            for_step(s + 1, (1, 2, 3), "start")
        if kind == "mid":
            for_step(s + 2, (0,), "start")

            @pl.when(s == NG - 3)
            def _():
                xcopy_b().start()

        for b in range(B):
            q = q_scr[b * SQ:(b + 1) * SQ, :]
            qs = jnp.concatenate([q[:, h * DH:(h + 1) * DH] for h in range(HG)], axis=0)
            s_scr[b] = lax.dot_general(qs, k_buf[slot, b], (((1,), (1,)), ((), ())),
                                       preferred_element_type=jnp.float32)

        for b in range(B):
            sc = jnp.where(mask, s_scr[b], -jnp.inf)
            m = jnp.max(sc, axis=-1, keepdims=True)
            p = jnp.exp((sc - m) * SCALE)
            l = jnp.sum(p, axis=-1, keepdims=True)
            r = pl.reciprocal(l, approx=True)
            r = r * (2.0 - l * r)
            p_scr[b] = (p * r).astype(jnp.bfloat16)

        if kind == "last":
            oproj(1 - slot, False)
        else:
            qproj_rows((s + 1) // NG, (s + 1) % 2, 0, M)

        for b in range(B):
            o = jnp.dot(p_scr[b], v_buf[slot, b], preferred_element_type=jnp.float32).astype(jnp.bfloat16)
            for h in range(HG):
                o_scr[slot, b * SQ:(b + 1) * SQ, h * DH:(h + 1) * DH] = o[h * SQ:(h + 1) * SQ, :]

        if kind == "mid":
            oproj(slot, g == 0)
        elif kind == "last":
            for c in range(OCH):
                rows = pl.ds(c * OR, OR)
                stage[1, rows, :] = (acc[rows, :] + jnp.dot(o_scr[slot, rows, :], wo_buf[slot],
                                                            preferred_element_type=jnp.float32)
                                     ).astype(stage.dtype)
                ochunk_b(c).start()
            ocopy_a().wait()
            for c in range(OCH):
                ochunk_b(c).wait()

    @pl.when(s < NSTEPS - 2)
    def _():
        step_body("mid")

    @pl.when(s == NSTEPS - 2)
    def _():
        step_body("penult")

    @pl.when(s == NSTEPS - 1)
    def _():
        step_body("last")

    @pl.when(s == NG - 1)
    def _():
        stage[0] = acc[...].astype(stage.dtype)
        ocopy_a().start()


@jax.jit
def pallas_concat_heads__mha_block_cached__mha_block_cached__near_ridge_kernel(
    A_x: jax.Array,
    A_k_cache: jax.Array,
    A_v_cache: jax.Array,
    A_wq: jax.Array,
    A_wo: jax.Array,
    B_x: jax.Array,
    B_k_cache: jax.Array,
    B_v_cache: jax.Array,
    B_wq: jax.Array,
    B_wo: jax.Array,
):
    def prep(x, k, v, wq, wo):
        return (x.reshape(M, D),
                k.reshape(B, NG, HG * SK, DH),
                v.reshape(B, NG, HG * SK, DH),
                wq, wo)

    args = prep(A_x, A_k_cache, A_v_cache, A_wq, A_wo) + prep(B_x, B_k_cache, B_v_cache, B_wq, B_wo)
    bf = jnp.bfloat16
    out = pl.pallas_call(
        _kernel,
        grid=(NSTEPS,),
        in_specs=[pl.BlockSpec(memory_space=pl.ANY)] * 10,
        out_specs=pl.BlockSpec(memory_space=pl.ANY),
        out_shape=jax.ShapeDtypeStruct((M, 2 * D), bf),
        scratch_shapes=[
            pltpu.VMEM((2, M, D), bf),
            pltpu.VMEM((2, D, GW), bf),
            pltpu.VMEM((2, GW, D), bf),
            pltpu.VMEM((2, B, HG * SK, DH), bf),
            pltpu.VMEM((2, B, HG * SK, DH), bf),
            pltpu.VMEM((M, GW), bf),
            pltpu.VMEM((2, M, GW), bf),
            pltpu.VMEM((M, D), jnp.float32),
            pltpu.VMEM((B, HG * SQ, HG * SK), jnp.float32),
            pltpu.VMEM((B, HG * SQ, HG * SK), bf),
            pltpu.VMEM((2, M, D), bf),
            pltpu.SemaphoreType.DMA((4, 2)),
            pltpu.SemaphoreType.DMA((XCH + 1,)),
            pltpu.SemaphoreType.DMA((OCH + 1,)),
        ],
        compiler_params=pltpu.CompilerParams(
            dimension_semantics=("arbitrary",),
            vmem_limit_bytes=64 * 1024 * 1024,
        ),
    )(*args)
    return out.reshape(B, SQ, 2 * D)
```

```python
import jax
import jax.numpy as jnp
from jax import lax
import jax.experimental.pallas as pl
import jax.experimental.pallas.tpu as pltpu

B, SQ, D = 32, 32, 640
H, SK, DH = 32, 32, 128
HG = 4
NG = H // HG
GW = HG * DH
M = B * SQ
NSTEPS = 2 * NG
SCALE = DH ** -0.5
XCH = 4
XR = M // XCH
OCH = 4
OR = M // OCH


def _kernel(xa, ka, va, wqa, woa, xb, kb, vb, wqb, wob,
            out_hbm,
            x_buf, wq_buf, wo_buf, k_buf, v_buf, q_scr, o_scr, acc, s_scr, p_scr, stage,
            sems, xsems, osems):
    s = pl.program_id(0)
    g = s % NG
    slot = s % 2
    refs = ((xa, ka, va, wqa, woa), (xb, kb, vb, wqb, wob))

    def cp(idx, branch, grp, sl):
        _, k, v, wq, wo = refs[branch]
        off = pl.multiple_of(grp * GW, GW)
        if idx == 0:
            return pltpu.make_async_copy(wq.at[:, pl.ds(off, GW)], wq_buf.at[sl], sems.at[0, sl])
        if idx == 1:
            return pltpu.make_async_copy(k.at[:, grp], k_buf.at[sl], sems.at[1, sl])
        if idx == 2:
            return pltpu.make_async_copy(v.at[:, grp], v_buf.at[sl], sems.at[2, sl])
        return pltpu.make_async_copy(wo.at[pl.ds(off, GW), :], wo_buf.at[sl], sems.at[3, sl])

    def start_step(t, idxs):
        for branch in range(2):
            @pl.when(t // NG == branch)
            def _():
                for idx in idxs:
                    cp(idx, branch, t % NG, t % 2).start()

    def wait_buf(idx, sl):
        buf = (wq_buf, k_buf, v_buf, wo_buf)[idx]
        pltpu.make_async_copy(buf.at[sl], buf.at[sl], sems.at[idx, sl]).wait()

    def xcopy_b():
        return pltpu.make_async_copy(xb, x_buf.at[1], xsems.at[XCH])

    def xchunk(c):
        return pltpu.make_async_copy(xa.at[pl.ds(c * XR, XR), :], x_buf.at[0, pl.ds(c * XR, XR), :],
                                     xsems.at[c])

    def ocopy_a():
        return pltpu.make_async_copy(stage.at[0], out_hbm.at[:, pl.ds(0, D)], osems.at[OCH])

    def ochunk_b(c):
        return pltpu.make_async_copy(stage.at[1, pl.ds(c * OR, OR), :],
                                     out_hbm.at[pl.ds(c * OR, OR), pl.ds(D, D)], osems.at[c])

    def qproj_rows(t_br, t_slot, r0, nrows):
        q_scr[pl.ds(r0, nrows), :] = jnp.dot(
            x_buf[t_br, pl.ds(r0, nrows), :], wq_buf[t_slot],
            preferred_element_type=jnp.float32).astype(jnp.bfloat16)

    def oproj(sl, first):
        prev = jnp.where(first, 0.0, acc[...])
        acc[...] = prev + jnp.dot(o_scr[sl], wo_buf[sl], preferred_element_type=jnp.float32)

    @pl.when(s == 0)
    def _():
        cp(0, 0, 0, 0).start()
        xchunk(0).start()
        cp(0, 0, 0, 0).wait()
        xchunk(0).wait()
        for c in range(1, XCH):
            xchunk(c).start()
        later = [cp(1, 0, 0, 0), cp(0, 0, 1, 1), cp(2, 0, 0, 0), cp(3, 0, 0, 0)]
        for c in range(XCH):
            if c > 0:
                xchunk(c).wait()
                later[c - 1].start()
            qproj_rows(0, 0, c * XR, XR)
        for l in later[XCH - 1:]:
            l.start()

    @pl.when(s == NG - 1)
    def _():
        xcopy_b().wait()

    row_h = lax.broadcasted_iota(jnp.int32, (HG * SQ, HG * SK), 0) // SQ
    col_h = lax.broadcasted_iota(jnp.int32, (HG * SQ, HG * SK), 1) // SK
    mask = row_h == col_h

    def step_body(kind):
        wait_buf(1, slot)
        if kind != "last":
            wait_buf(0, 1 - slot)
        if kind != "first":
            wait_buf(2, slot)
            wait_buf(3, slot)

        if kind != "last":
            start_step(s + 1, (1, 2, 3))
        if kind in ("first", "mid"):
            start_step(s + 2, (0,))

            @pl.when(s == NG - 3)
            def _():
                xcopy_b().start()

        for b in range(B):
            q = q_scr[b * SQ:(b + 1) * SQ, :]
            qs = jnp.concatenate([q[:, h * DH:(h + 1) * DH] for h in range(HG)], axis=0)
            s_scr[b] = lax.dot_general(qs, k_buf[slot, b], (((1,), (1,)), ((), ())),
                                       preferred_element_type=jnp.float32)

        for b in range(B):
            sc = jnp.where(mask, s_scr[b], -jnp.inf)
            m = jnp.max(sc, axis=-1, keepdims=True)
            p = jnp.exp((sc - m) * SCALE)
            l = jnp.sum(p, axis=-1, keepdims=True)
            r = pl.reciprocal(l, approx=True)
            r = r * (2.0 - l * r)
            p_scr[b] = (p * r).astype(jnp.bfloat16)

        if kind == "last":
            oproj(1 - slot, False)
        else:
            qproj_rows((s + 1) // NG, (s + 1) % 2, 0, M)

        if kind == "first":
            wait_buf(2, slot)
            wait_buf(3, slot)
        for b in range(B):
            o = jnp.dot(p_scr[b], v_buf[slot, b], preferred_element_type=jnp.float32).astype(jnp.bfloat16)
            for h in range(HG):
                o_scr[slot, b * SQ:(b + 1) * SQ, h * DH:(h + 1) * DH] = o[h * SQ:(h + 1) * SQ, :]

        if kind in ("first", "mid"):
            oproj(slot, g == 0)
        elif kind == "last":
            for c in range(OCH):
                rows = pl.ds(c * OR, OR)
                stage[1, rows, :] = (acc[rows, :] + jnp.dot(o_scr[slot, rows, :], wo_buf[slot],
                                                            preferred_element_type=jnp.float32)
                                     ).astype(stage.dtype)
                ochunk_b(c).start()
            ocopy_a().wait()
            for c in range(OCH):
                ochunk_b(c).wait()

    @pl.when(s == 0)
    def _():
        step_body("first")

    @pl.when(jnp.logical_and(s > 0, s < NSTEPS - 2))
    def _():
        step_body("mid")

    @pl.when(s == NSTEPS - 2)
    def _():
        step_body("penult")

    @pl.when(s == NSTEPS - 1)
    def _():
        step_body("last")

    @pl.when(s == NG - 1)
    def _():
        stage[0] = acc[...].astype(stage.dtype)
        ocopy_a().start()


@jax.jit
def pallas_concat_heads__mha_block_cached__mha_block_cached__near_ridge_kernel(
    A_x: jax.Array,
    A_k_cache: jax.Array,
    A_v_cache: jax.Array,
    A_wq: jax.Array,
    A_wo: jax.Array,
    B_x: jax.Array,
    B_k_cache: jax.Array,
    B_v_cache: jax.Array,
    B_wq: jax.Array,
    B_wo: jax.Array,
):
    def prep(x, k, v, wq, wo):
        return (x.reshape(M, D),
                k.reshape(B, NG, HG * SK, DH),
                v.reshape(B, NG, HG * SK, DH),
                wq, wo)

    args = prep(A_x, A_k_cache, A_v_cache, A_wq, A_wo) + prep(B_x, B_k_cache, B_v_cache, B_wq, B_wo)
    bf = jnp.bfloat16
    out = pl.pallas_call(
        _kernel,
        grid=(NSTEPS,),
        in_specs=[pl.BlockSpec(memory_space=pl.ANY)] * 10,
        out_specs=pl.BlockSpec(memory_space=pl.ANY),
        out_shape=jax.ShapeDtypeStruct((M, 2 * D), bf),
        scratch_shapes=[
            pltpu.VMEM((2, M, D), bf),
            pltpu.VMEM((2, D, GW), bf),
            pltpu.VMEM((2, GW, D), bf),
            pltpu.VMEM((2, B, HG * SK, DH), bf),
            pltpu.VMEM((2, B, HG * SK, DH), bf),
            pltpu.VMEM((M, GW), bf),
            pltpu.VMEM((2, M, GW), bf),
            pltpu.VMEM((M, D), jnp.float32),
            pltpu.VMEM((B, HG * SQ, HG * SK), jnp.float32),
            pltpu.VMEM((B, HG * SQ, HG * SK), bf),
            pltpu.VMEM((2, M, D), bf),
            pltpu.SemaphoreType.DMA((4, 2)),
            pltpu.SemaphoreType.DMA((XCH + 1,)),
            pltpu.SemaphoreType.DMA((OCH + 1,)),
        ],
        compiler_params=pltpu.CompilerParams(
            dimension_semantics=("arbitrary",),
            vmem_limit_bytes=64 * 1024 * 1024,
        ),
    )(*args)
    return out.reshape(B, SQ, 2 * D)
```
